```python
import os as _os
_os.environ.setdefault("JAX_PLATFORMS", "cpu")
import jax
import jax.numpy as jnp

def _softmax(x, axis=-1):
    return jax.nn.softmax(x, axis=axis)
def _gelu(x):
    return jax.nn.gelu(x, approximate=True)
def _silu(x):
    return jax.nn.silu(x)
def _sigmoid(x):
    return jax.nn.sigmoid(x)
def _layernorm(x, axis=-1, eps=1e-5):
    m = jnp.mean(x, axis=axis, keepdims=True)
    v = jnp.var(x, axis=axis, keepdims=True)
    return (x - m) / jnp.sqrt(v + eps)
def _scatter_add(tgt, idx, src, axis=0):
    return tgt.at[idx].add(src)
def _segment_sum(src, seg, n):
    return jax.ops.segment_sum(src, seg, n)
class _Rng:
    def __init__(self, key):
        self._k = key
    def _next(self):
        self._k, sub = jax.random.split(self._k)
        return sub
    def normal(self, shape):
        return jax.random.normal(self._next(), shape, dtype=jnp.bfloat16)
    def randint(self, lo, hi, shape):
        return jax.random.randint(self._next(), shape, lo, hi, dtype=jnp.int32)
    def uniform(self, shape, lo=0.0, hi=1.0):
        return jax.random.uniform(self._next(), shape, jnp.bfloat16, lo, hi)
    def permutation(self, n):
        return jax.random.permutation(self._next(), n)


kernel_name = 'parallel_sum__mha_block_cached__dense_activation_mish__decode'

def setup_inputs():
    _rng = _Rng(jax.random.key(int.from_bytes(__import__("os").urandom(4), "little")))
    _w = (lambda a: (lambda t: t.astype(jnp.bfloat16) if jnp.issubdtype(t.dtype, jnp.floating) else t)(jnp.asarray(a)))
    def _A_setup():
        B, Sq, D = 1, 1, 448
        H, Sk, Dh = 16, 16384, 256
        return {
            "x": _w((lambda *s: _rng.normal(s) * 0.05)(B, Sq, D)),
            "k_cache": _w((lambda *s: _rng.normal(s) * 1.6)(B, H, Sk, Dh)),
            "v_cache": _w((lambda *s: _rng.normal(s) * 0.8)(B, H, Sk, Dh)),
            "wq": _w((lambda *s: _rng.normal(s) * 1.6)(D, H * Dh) * (D ** -0.5)),
            "wo": _w((lambda *s: _rng.normal(s) * 0.8)(H * Dh, D) * ((H * Dh) ** -0.5)),
        }
    _A_in = _A_setup()

    def _B_setup():
        B, S, D, F = 1, 1, 448, 1792
        return {
            "x": _w((lambda *s: _rng.normal(s) * 0.05)(B, S, D)),
            "w1": _w((lambda *s: _rng.normal(s) * 0.8)(D, F) * (D ** -0.5)),
            "b1": _w((lambda *s: _rng.normal(s) * 0.05)(F)),
            "w2": _w((lambda *s: _rng.normal(s) * 0.05)(F, D) * (F ** -0.5)),
        }
    _B_in = _B_setup()

    return {
        "A_x": _A_in["x"],
        "A_k_cache": _A_in["k_cache"],
        "A_v_cache": _A_in["v_cache"],
        "A_wq": _A_in["wq"],
        "A_wo": _A_in["wo"],
        "B_x": _B_in["x"],
        "B_w1": _B_in["w1"],
        "B_b1": _B_in["b1"],
        "B_w2": _B_in["w2"],
    }

def reference(A_x, A_k_cache, A_v_cache, A_wq, A_wo, B_x, B_w1, B_b1, B_w2):
    def _A_ref(x, k_cache, v_cache, wq, wo):
        B, Sq, D = x.shape
        H, Dh = 16, 256
        q = (lambda x, *d: x.transpose(*d))((x @ wq).reshape(B, Sq, H, Dh), 0, 2, 1, 3)
        scores = jnp.einsum("bhqd,bhkd->bhqk", q, k_cache) * (Dh ** -0.5)
        p = _softmax(scores, axis=-1)
        o = jnp.einsum("bhqk,bhkd->bhqd", p, v_cache)
        return (lambda x, *d: x.transpose(*d))(o, 0, 2, 1, 3).reshape(B, Sq, H * Dh) @ wo

    def _B_ref(x, w1, b1, w2):
        h = jnp.einsum("bsd,df->bsf", x, w1) + b1
        sp = jnp.log1p(jnp.exp(-jnp.abs(h))) + jnp.where(h > 0, h, jnp.zeros_like(h))
        act = h * jnp.tanh(sp)
        return jnp.einsum("bsf,fd->bsd", act, w2)

    x = A_x
    xn = _layernorm(x, axis=-1)
    return x + _A_ref(xn, A_k_cache, A_v_cache, A_wq, A_wo) + _B_ref(xn, B_w1, B_b1, B_w2)
```

```python
import numpy as np
import jax, jax.numpy as jnp
from jax import lax
import jax.experimental.pallas as pl
import jax.experimental.pallas.tpu as pltpu
bf = jnp.bfloat16
f32 = jnp.float32
D, H, SK, DH, F = 448, 16, 16384, 256, 1792
NT = (((1,), (1,)), ((), ()))

def make(seg=16, piece=32, hps=4, lag=2, wstride=9, flags=None, out_vmem=False, mlp_pos="start", sub=4, prios=(0, 1)):
    L = SK // seg
    T = seg * piece
    nrounds = L // piece
    spr = H // hps
    nsteps = nrounds * spr
    nslots = lag + 1
    def f(A_x, A_k, A_v, A_wq, A_wo, B_x, B_w1, B_b1, B_w2):
        def kern(x_h, k_h, v_h, wq_h, wo_h, w1_h, b1_h, w2_h, o_h,
                 kv, s_ref, wq, wo, w1, w2, xs, bs, os, q_ref, kv_sem, w_sem):
            def kv_pieces(src, i, slot):
                r = lax.shift_right_logical(i, int(np.log2(spr))) if not isinstance(i, int) else i // spr
                g0 = (i & (spr - 1)) * (hps * seg)
                row = r * piece if isinstance(r, int) else pl.multiple_of(r * piece, piece)
                return [(lambda n=n: pltpu.make_async_copy(src.at[g0 + n, pl.ds(row, piece)], kv.at[slot, pl.ds(n * piece, piece)], kv_sem.at[slot])) for n in range(hps * seg)]
            def kv_wait(slot):
                pltpu.make_async_copy(kv.at[slot], kv.at[slot], kv_sem.at[slot]).wait()
            def w_pieces(src, dst, c0, cn, sem, r0=0, rn=D):
                n = rn // 8
                st = wstride if np.gcd(wstride, n) == 1 else 1
                idx = [(p * st) % n for p in range(n)]
                return [(lambda p=p: pltpu.make_async_copy(src.at[pl.ds(r0 + 8 * p, 8), pl.ds(c0, cn)], dst.at[pl.ds(r0 + 8 * p, 8), pl.ds(c0, cn)], w_sem.at[sem])) for p in idx]
            def w_wait(dst, c0, cn, sem, r0=0, rn=D):
                v = dst.at[pl.ds(r0, rn), pl.ds(c0, cn)]
                pltpu.make_async_copy(v, v, w_sem.at[sem]).wait()
            def issue(pieces, part=0, nparts=1):
                lo, hi = len(pieces) * part // nparts, len(pieces) * (part + 1) // nparts
                for n in range(lo, hi): pieces[n]().start(priority=prios[n % len(prios)])

            cx = pltpu.make_async_copy(x_h, xs, w_sem.at[0]); cx.start()
            cb = pltpu.make_async_copy(b1_h, bs, w_sem.at[1]); cb.start()
            head = [w_pieces(wq_h, wq, 1024 * j, 1024, 2 + j) for j in range(4)]
            head += [w_pieces(w1_h, w1, 896 * j, 896, 6 + j) for j in range(2)]
            head += [w_pieces(w2_h, w2, 896 * j, 896, 8 + j) for j in range(2)]
            head += [kv_pieces(k_h, j, j) for j in range(lag)]
            rows_last = [(0, 128), (128, 128), (256, 128), (384, 64)]
            tail = [w_pieces(wo_h, wo, 1024 * j, 1024, 10 + j) for j in range(3)]
            tail += [sum((w_pieces(wo_h, wo, 3072, 1024, 13 + m, r0, rn) for m, (r0, rn) in enumerate(rows_last)), [])]
            tail += [[]] * lag
            for g in range(lag): issue(head[g])

            cx.wait()
            x = xs[0].astype(f32)
            mu = jnp.mean(x, axis=-1, keepdims=True)
            xc = x - mu
            var = jnp.mean(xc * xc, axis=-1, keepdims=True)
            xn = jnp.broadcast_to(xc * lax.rsqrt(var + 1e-5), (H, D)).astype(bf)
            row128 = lax.broadcasted_iota(jnp.int32, (H, 128), 0)
            row256 = lax.broadcasted_iota(jnp.int32, (H, DH), 0)
            rowT = lax.broadcasted_iota(jnp.int32, (H, T), 0)
            q = jnp.zeros((H, DH), f32)
            for j in range(4):
                w_wait(wq, 1024 * j, 1024, 2 + j)
                for u in range(8):
                    issue(head[j + lag], u, 8)
                    if u % 2 == 0:
                        h = 4 * j + u // 2
                        q = jnp.where(row256 == h, jnp.dot(xn, wq[:, DH * h:DH * (h + 1)], preferred_element_type=f32), q)
            q_ref[...] = q.astype(bf)
            hid = jnp.zeros((H, 128), f32)
            for j in range(2):
                w_wait(w1, 896 * j, 896, 6 + j)
                for u in range(7):
                    issue(head[4 + j + lag], u, 7)
                    c = 7 * j + u
                    hid = jnp.where(row128 == c, jnp.dot(xn, w1[:, 128 * c:128 * (c + 1)], preferred_element_type=f32), hid)
            cb.wait()
            hid = hid + jnp.concatenate([bs[...].astype(f32), jnp.zeros((H - F // 128, 128), f32)], axis=0)
            sp = jnp.log1p(jnp.exp(-jnp.abs(hid))) + jnp.where(hid > 0, hid, 0.0)
            act = (hid * jnp.tanh(sp))
            y = jnp.zeros((H, D), f32)
            for j in range(2):
                w_wait(w2, 896 * j, 896, 8 + j)
                for u in range(7):
                    issue(head[6 + j + lag], u, 7)
                    c = 7 * j + u
                    y = y + lax.dot_general(jnp.where(row128 == c, act, 0.0).astype(bf), w2[:, 128 * c:128 * (c + 1)], NT, preferred_element_type=f32)
            nxt = lambda s: jnp.where(s == nslots - 1, 0, s + 1)
            prv = lambda s: jnp.where(s == 0, nslots - 1, s - 1)
            def kstep(i, carry, src, j):
                slot, s, m = carry
                kv_wait(slot)
                pieces = kv_pieces(src, j, prv(slot))
                qb = q_ref[...]
                h0 = (i & (spr - 1)) * hps
                for u in range(hps):
                    parts = []
                    for t in range(sub):
                        issue(pieces, u * sub + t, hps * sub)
                        n = T // sub
                        parts.append(lax.dot_general(qb, kv[slot, pl.ds(u * T + t * n, n)], NT, preferred_element_type=f32))
                    s = jnp.where(rowT == h0 + u, jnp.concatenate(parts, axis=1), s)
                s_ref[lax.shift_right_logical(i, int(np.log2(spr)))] = s
                return nxt(slot), s, jnp.maximum(m, s)
            ninf = jnp.full((H, T), -jnp.inf, f32)
            c = (jnp.int32(0), ninf, ninf)
            c = lax.fori_loop(0, nsteps - lag, lambda i, c: kstep(i, c, k_h, i + lag), c)
            c = lax.fori_loop(nsteps - lag, nsteps, lambda i, c: kstep(i, c, v_h, i + lag - nsteps), c)
            slot, _, m = c
            m = jnp.max(m, axis=1, keepdims=True)
            def vstep(i, carry, pieces_fn):
                slot, l, acc = carry
                kv_wait(slot)
                pieces = pieces_fn(prv(slot))
                r = lax.shift_right_logical(i, int(np.log2(spr))) if not isinstance(i, int) else i // spr
                p = jnp.exp((s_ref[r] - m) * (DH ** -0.5))
                pb = p.astype(bf)
                h0 = (i & (spr - 1)) * hps
                for u in range(hps):
                    a = None
                    for t in range(sub):
                        issue(pieces, u * sub + t, hps * sub)
                        n = T // sub
                        d = jnp.dot(pb[:, t * n:(t + 1) * n], kv[slot, pl.ds(u * T + t * n, n)], preferred_element_type=f32)
                        a = d if a is None else a + d
                    acc = acc + jnp.where(row256 == h0 + u, a, 0.0)
                l = l + jnp.where((rowT >= h0) & (rowT < h0 + hps), p, 0.0)
                return nxt(slot), l, acc
            c = (slot, jnp.zeros((H, T), f32), jnp.zeros((H, DH), f32))
            c = lax.fori_loop(0, nsteps - lag, lambda i, c: vstep(i, c, lambda sl: kv_pieces(v_h, i + lag, sl)), c)
            for g in range(lag):
                c = vstep(nsteps - lag + g, c, lambda sl: tail[g])
            _, l, acc = c
            o = acc / jnp.sum(l, axis=1, keepdims=True)
            for j in range(3):
                w_wait(wo, 1024 * j, 1024, 10 + j)
                for u in range(8):
                    issue(tail[j + lag], u, 8)
                    if u % 2 == 0:
                        h = 4 * j + u // 2
                        y = y + lax.dot_general(jnp.where(row256 == h, o, 0.0).astype(bf), wo[:, DH * h:DH * (h + 1)], NT, preferred_element_type=f32)
            olast = jnp.concatenate([jnp.where(row256 == h, o, 0.0).astype(bf) for h in range(12, 16)], axis=1)
            parts = []
            for mi, (r0, rn) in enumerate(rows_last):
                w_wait(wo, 3072, 1024, 13 + mi, r0, rn)
                parts.append(lax.dot_general(olast, wo[r0:r0 + rn, 3072:4096], NT, preferred_element_type=f32))
            y = y + jnp.concatenate(parts, axis=1)
            out = (x + jnp.sum(y, axis=0, keepdims=True)).astype(bf)
            if out_vmem:
                o_h[0] = out
            else:
                os[0] = out
                co = pltpu.make_async_copy(os, o_h, w_sem.at[0]); co.start(); co.wait()
        hbm = pl.BlockSpec(memory_space=pltpu.HBM)
        return pl.pallas_call(kern, out_shape=jax.ShapeDtypeStruct((1, 1, D), bf), in_specs=[hbm]*8,
            out_specs=pl.BlockSpec(memory_space=pltpu.VMEM) if out_vmem else hbm,
            scratch_shapes=[pltpu.VMEM((nslots, hps * T, DH), bf), pltpu.VMEM((nrounds, H, T), f32),
                            pltpu.VMEM((D, H * DH), bf), pltpu.VMEM((D, H * DH), bf), pltpu.VMEM((D, F), bf), pltpu.VMEM((D, F), bf),
                            pltpu.VMEM((1, 1, D), bf), pltpu.VMEM((F // 128, 128), bf), pltpu.VMEM((1, 1, D), bf), pltpu.VMEM((H, DH), bf),
                            pltpu.SemaphoreType.DMA((nslots,)), pltpu.SemaphoreType.DMA((17,))],
            compiler_params=pltpu.CompilerParams(vmem_limit_bytes=64*2**20, disable_bounds_checks=True, flags=flags),
            name="k2",
        )(A_x, A_k.reshape(H * seg, L, DH), A_v.reshape(H * seg, L, DH), A_wq, A_wo.T, B_w1, B_b1.reshape(F // 128, 128), B_w2.T)
    return f


@jax.jit
def pallas_parallel_sum__mha_block_cached__dense_activation_mish__decode_kernel(A_x, A_k_cache, A_v_cache, A_wq, A_wo, B_x, B_w1, B_b1, B_w2):
    return make(hps=2, lag=3)(A_x, A_k_cache, A_v_cache, A_wq, A_wo, B_x, B_w1, B_b1, B_w2)
```

```python
import jax
import jax.numpy as jnp
from jax import lax
import jax.experimental.pallas as pl
import jax.experimental.pallas.tpu as pltpu

_H, _DH = 16, 256
_LANES = 128
_EPS = 1e-5

_SEGS = 16
_PIECE = 32
_TILES = _SEGS * _PIECE // _LANES
_RING = 8
_AHEAD = 90
_SKEW = 10
_WROWS = 8
_WCOLS = 1024
_DRAIN = 24

_NT = (((1,), (1,)), ((), ()))


def _dot(a, b):
    return jnp.dot(a, b, preferred_element_type=jnp.float32)


def _dot_nt(a, b):
    return lax.dot_general(a, b, _NT, preferred_element_type=jnp.float32)


def _spread(n, step=8):
    return [a + b for a in range(step) for b in range(0, n, step) if a + b < n]


def _kernel(x_hbm, k_hbm, v_hbm, wq_hbm, wot_hbm, w1_hbm, b1_hbm, w2t_hbm, out_hbm,
            kv, scores, q_ref, wq, wot, w1, w2t, x_ref, b1_ref, out_ref,
            kv_sem, wq_sem, wo_sem, misc_sem):
    f32, bf16 = jnp.float32, jnp.bfloat16
    d, ff = w1.shape
    n_blocks = scores.shape[0] * _H
    n_inner = n_blocks - pl.cdiv(_AHEAD, _SEGS)
    w_tiles = d // _WROWS
    w_groups = _H * _DH // _WCOLS
    heads_per_group = _H // w_groups

    def round_of(blk):
        if isinstance(blk, int):
            return blk // _H
        return lax.shift_right_logical(blk, _H.bit_length() - 1)

    def kv_start(src, blk, c):
        rnd = round_of(blk)
        row = rnd * _PIECE
        if not isinstance(blk, int):
            row = pl.multiple_of(row, _PIECE)
        odd = c % 2
        head = (blk + _SKEW * odd) & (_H - 1)
        seg = (head * _SEGS + ((rnd + odd) & 1)) + (c - odd)
        slot = blk & (_RING - 1)
        pltpu.make_async_copy(
            src.at[seg, pl.ds(row, _PIECE)],
            kv.at[slot, pl.ds(c * _PIECE, _PIECE)],
            kv_sem.at[slot],
        ).start(priority=odd)

    def kv_wait(blk):
        slot = blk & (_RING - 1)
        pltpu.make_async_copy(kv.at[slot], kv.at[slot], kv_sem.at[slot]).wait()

    def kv_tile(blk, t):
        return kv[blk & (_RING - 1), pl.ds(t * _LANES, _LANES)]

    def w_copy(src, dst, sem, row, col, rows=_WROWS, cols=_WCOLS):
        where = (pl.ds(row, rows), pl.ds(col, cols))
        return pltpu.make_async_copy(src.at[where], dst.at[where], sem)

    def step(start, tasks, pieces=_SEGS):
        for part in range(4):
            for p in range(pieces * part // 4, pieces * (part + 1) // 4):
                start(p + _AHEAD)
            for task in tasks[part::4]:
                task()

    def share(tasks, blk):
        j, n = blk - n_inner, n_blocks - n_inner
        return tasks[len(tasks) * j // n:len(tasks) * (j + 1) // n]

    row = lax.broadcasted_iota(jnp.int32, (_H, _LANES), 0)
    col = lax.broadcasted_iota(jnp.int32, (_H, _LANES), 1)
    row_dh = lax.broadcasted_iota(jnp.int32, (_H, _DH), 0)
    owner = (row - _SKEW * ((col >> (_PIECE.bit_length() - 1)) & 1)) & (_H - 1)

    wq_pieces = [(_WROWS * p, _WCOLS * g) for g in range(w_groups) for p in _spread(w_tiles)]

    def wq_copy(n):
        return w_copy(wq_hbm, wq, wq_sem.at[n // _SEGS], *wq_pieces[n])

    def start_head(n):
        if n < len(wq_pieces):
            wq_copy(n).start(priority=n % 2)
        else:
            kv_start(k_hbm, *divmod(n - len(wq_pieces), _SEGS))

    x_copy = pltpu.make_async_copy(x_hbm, x_ref, misc_sem.at[0])
    b1_copy = pltpu.make_async_copy(b1_hbm, b1_ref, misc_sem.at[1])
    x_copy.start()
    for n in range(0, 36):
        start_head(n)
    x_copy.wait()
    b1_copy.start()
    for n in range(36, 64):
        start_head(n)
    x = x_ref[0].astype(f32)
    centered = x - jnp.mean(x, axis=-1, keepdims=True)
    var = jnp.mean(centered * centered, axis=-1, keepdims=True)
    xn = jnp.broadcast_to(centered * lax.rsqrt(var + _EPS), (_H, d)).astype(bf16)
    b1_copy.wait()
    for n in range(64, _AHEAD):
        start_head(n)

    q = [jnp.zeros((_H, _DH), f32)]

    def project_q(h):
        q[0] = jnp.where(row_dh == h, _dot(xn, wq[:, _DH * h:_DH * (h + 1)]), q[0])

    done = 0
    for first in range(0, len(wq_pieces), _SEGS):
        for n in range(first, first + _SEGS):
            wq_copy(n).wait()
        landed = heads_per_group * ((first + _SEGS) // w_tiles)
        upto = landed if landed == _H else min(landed, done + 2)
        step(lambda p: start_head(first + p),
             [lambda h=h: project_q(h) for h in range(done, upto)])
        done = upto
    q_ref[...] = q[0].astype(bf16)

    def score_block(blk, carry, start, extra=()):
        s, m = list(carry[0]), [carry[1]]
        kv_wait(blk)
        qs = q_ref[...]

        def tile(t):
            s[t] = jnp.where(owner == (blk & (_H - 1)), _dot_nt(qs, kv_tile(blk, t)), s[t])
            scores[round_of(blk), t] = s[t]
            m[0] = jnp.maximum(m[0], s[t])

        step(start, [lambda t=t: tile(t) for t in range(_TILES)] + list(extra))
        return tuple(s), m[0]

    def ahead(src, blk):
        return lambda p: kv_start(src, blk + p // _SEGS, p % _SEGS)

    def start_mlp_weights(n):
        r = pl.multiple_of(lax.shift_right_logical(n, 1) * _WROWS, _WROWS)
        c = pl.multiple_of((n & 1) * (ff // 2), _LANES)
        w_copy(w1_hbm, w1, misc_sem.at[0], r, c, cols=ff // 2).start(priority=0)
        w_copy(w2t_hbm, w2t, misc_sem.at[1], r, c, cols=ff // 2).start(priority=1)

    lowest = jnp.full((_H, _LANES), -jnp.inf, f32)
    carry = lax.fori_loop(
        0, 2 * w_tiles,
        lambda b, c: score_block(b, c, ahead(k_hbm, b), [lambda: start_mlp_weights(b)]),
        ((lowest,) * _TILES, lowest))
    carry = lax.fori_loop(
        2 * w_tiles, n_inner, lambda b, c: score_block(b, c, ahead(k_hbm, b)), carry)
    pltpu.make_async_copy(w1, w1, misc_sem.at[0]).wait()
    pltpu.make_async_copy(w2t, w2t, misc_sem.at[1]).wait()

    hidden = [jnp.zeros((_H, _LANES), f32)]

    def mlp_in(c):
        h = _dot(xn, w1[:, _LANES * c:_LANES * (c + 1)])
        hidden[0] = jnp.where(row == c, h, hidden[0])

    def start_k_then_v(n):
        blk, c = divmod(n, _SEGS)
        kv_start(k_hbm if blk < n_blocks else v_hbm, blk % n_blocks, c)

    tasks = [lambda c=c: mlp_in(c) for c in range(ff // _LANES)]
    for b in range(n_inner, n_blocks):
        carry = score_block(b, carry, lambda p: start_k_then_v(b * _SEGS + p), share(tasks, b))
    row_max = jnp.max(carry[1], axis=1, keepdims=True)

    bias = jnp.concatenate(
        [b1_ref[...].astype(f32), jnp.zeros((_H - ff // _LANES, _LANES), f32)], axis=0)
    pre = hidden[0] + bias
    softplus = jnp.log1p(jnp.exp(-jnp.abs(pre))) + jnp.where(pre > 0, pre, 0.0)
    act = pre * jnp.tanh(softplus)

    def value_block(blk, carry, start, extra=()):
        denom, acc = carry[0], [carry[1]]
        p = []
        for t in range(_TILES):
            e = jnp.exp((scores[round_of(blk), t] - row_max) * (_DH ** -0.5))
            p.append(jnp.where(owner == (blk & (_H - 1)), e, 0.0))
            denom = denom + p[t]
        kv_wait(blk)

        def tile(t):
            acc[0] = acc[0] + _dot(p[t].astype(bf16), kv_tile(blk, t))

        step(start, [lambda t=t: tile(t) for t in range(_TILES)] + list(extra))
        return denom, acc[0]

    row_blocks = [(r, min(_LANES, d - r)) for r in range(0, d, _LANES)]
    wo_units = []
    for g in range(w_groups):
        if g < w_groups // 2:
            pieces = [(_WROWS * p, _WCOLS * g) for p in _spread(w_tiles)]
            wo_units += [(pieces[:16], None, []), (pieces[16:32], None, []),
                         (pieces[32:], None, [(g, i) for i in range(len(row_blocks))])]
            continue
        for blocks in ([0], [1], [2, 3]) if g < w_groups - 1 else ([0], [1], [2], [3]):
            pieces = [(row_blocks[i][0] + _WROWS * p, _WCOLS * g)
                      for i in blocks for p in _spread(row_blocks[i][1] // _WROWS)]
            region = (row_blocks[blocks[0]][0], _WCOLS * g, _WROWS * len(pieces))
            wo_units.append((pieces, region, [(g, i) for i in blocks]))
    wo_pieces = [(u, piece) for u, unit in enumerate(wo_units) for piece in unit[0]]

    def start_tail(n):
        if n < 0:
            kv_start(v_hbm, n_blocks + n // _SEGS, n % _SEGS)
        elif n < len(wo_pieces):
            u, piece = wo_pieces[n]
            late = n >= len(wo_pieces) - _DRAIN
            w_copy(wot_hbm, wot, wo_sem.at[u], *piece).start(priority=1 if late else n % 2)

    mlp = [jnp.zeros((_H, d), f32)]

    def mlp_out(c):
        lhs = jnp.where(row == c, act, 0.0).astype(bf16)
        mlp[0] = mlp[0] + _dot_nt(lhs, w2t[:, _LANES * c:_LANES * (c + 1)])

    carry = lax.fori_loop(
        0, n_inner, lambda b, c: value_block(b, c, ahead(v_hbm, b)),
        (jnp.zeros((_H, _LANES), f32), jnp.zeros((_H, _DH), f32)))
    tasks = [lambda c=c: mlp_out(c) for c in range(ff // _LANES)]
    for b in range(n_inner, n_blocks):
        carry = value_block(
            b, carry, lambda p: start_tail((b - n_blocks) * _SEGS + p), share(tasks, b))

    attn = carry[1] / jnp.sum(carry[0], axis=1, keepdims=True)
    attn_rows = [
        jnp.concatenate(
            [jnp.broadcast_to(attn[h:h + 1], (_H, _DH))
             for h in range(heads_per_group * g, heads_per_group * (g + 1))],
            axis=1).astype(bf16)
        for g in range(w_groups)]
    base = x + jnp.sum(mlp[0], axis=0, keepdims=True)
    out = [base[:, r:r + n] for r, n in row_blocks]

    def project_out(g, i):
        r, n = row_blocks[i]
        out[i] = out[i] + _dot_nt(attn_rows[g], wot[r:r + n, _WCOLS * g:_WCOLS * (g + 1)])[:1]

    first, todo = 0, []
    for u, (pieces, region, unlocked) in enumerate(wo_units):
        if region is None:
            for piece in pieces:
                w_copy(wot_hbm, wot, wo_sem.at[u], *piece).wait()
        else:
            w_copy(wot_hbm, wot, wo_sem.at[u], *region).wait()
        todo += unlocked
        now, todo = todo[:3], todo[3:]
        step(lambda p: start_tail(first + p),
             [lambda a=a: project_out(*a) for a in now], len(pieces))
        first += len(pieces)
    assert not todo

    out_ref[0] = jnp.concatenate(out, axis=1).astype(out_ref.dtype)
    out_copy = pltpu.make_async_copy(out_ref, out_hbm, misc_sem.at[0])
    out_copy.start()
    out_copy.wait()


@jax.jit
def pallas_parallel_sum__mha_block_cached__dense_activation_mish__decode_kernel(
    A_x: jax.Array,
    A_k_cache: jax.Array,
    A_v_cache: jax.Array,
    A_wq: jax.Array,
    A_wo: jax.Array,
    B_x: jax.Array,
    B_w1: jax.Array,
    B_b1: jax.Array,
    B_w2: jax.Array,
):
    del B_x
    d, ff = B_w1.shape
    seg_rows = A_k_cache.shape[2] // _SEGS
    dtype = A_x.dtype
    hbm = pl.BlockSpec(memory_space=pltpu.HBM)
    return pl.pallas_call(
        _kernel,
        out_shape=jax.ShapeDtypeStruct(A_x.shape, dtype),
        in_specs=[hbm] * 8,
        out_specs=hbm,
        scratch_shapes=[
            pltpu.VMEM((_RING, _SEGS * _PIECE, _DH), dtype),
            pltpu.VMEM((seg_rows // _PIECE, _TILES, _H, _LANES), jnp.float32),
            pltpu.VMEM((_H, _DH), jnp.bfloat16),
            pltpu.VMEM((d, _H * _DH), dtype),
            pltpu.VMEM((d, _H * _DH), dtype),
            pltpu.VMEM((d, ff), dtype),
            pltpu.VMEM((d, ff), dtype),
            pltpu.VMEM(A_x.shape, dtype),
            pltpu.VMEM((ff // _LANES, _LANES), dtype),
            pltpu.VMEM(A_x.shape, dtype),
            pltpu.SemaphoreType.DMA((_RING,)),
            pltpu.SemaphoreType.DMA((14,)),
            pltpu.SemaphoreType.DMA((13,)),
            pltpu.SemaphoreType.DMA((2,)),
        ],
        compiler_params=pltpu.CompilerParams(
            vmem_limit_bytes=32 * 2**20,
            disable_bounds_checks=True,
            disable_semaphore_checks=True,
        ),
    )(
        A_x,
        A_k_cache.reshape(_H * _SEGS, seg_rows, _DH),
        A_v_cache.reshape(_H * _SEGS, seg_rows, _DH),
        A_wq,
        A_wo.T,
        B_w1,
        B_b1.reshape(ff // _LANES, _LANES),
        B_w2.T,
    )
```

```python
import jax
import jax.numpy as jnp
from jax import lax
import jax.experimental.pallas as pl
import jax.experimental.pallas.tpu as pltpu

_H, _DH = 16, 256
_LANES = 128
_EPS = 1e-5

_SEGS = 16
_PIECE = 32
_ROUND = _H * _SEGS
_TILES = _SEGS * _PIECE // _LANES
_AHEAD = 92
_BURST = 8
_SKEW = 11
_WROWS = 8
_WCOLS = 1024
_DRAIN = 24

_NT = (((1,), (1,)), ((), ()))


def _dot(a, b):
    return jnp.dot(a, b, preferred_element_type=jnp.float32)


def _dot_nt(a, b):
    return lax.dot_general(a, b, _NT, preferred_element_type=jnp.float32)


def _spread(n, step=8):
    return [a + b for a in range(step) for b in range(0, n, step) if a + b < n]


def _kernel(x_hbm, k_hbm, v_hbm, wq_hbm, wot_hbm, w1_hbm, b1_hbm, w2t_hbm, out_hbm,
            kv, scores, q_ref, wq, wot, w1, w2t, x_ref, b1_ref, out_ref,
            kv_sem, wq_sem, wo_sem, misc_sem):
    f32, bf16 = jnp.float32, jnp.bfloat16
    d, ff = w1.shape
    last_round = scores.shape[0] - 1
    w_tiles = d // _WROWS
    w_groups = _H * _DH // _WCOLS
    heads_per_group = _H // w_groups

    def kv_start(src, rnd, n):
        rnd = rnd + n // _ROUND
        blk, c = divmod(n % _ROUND, _SEGS)
        first_row = rnd * _PIECE
        if not isinstance(rnd, int):
            first_row = pl.multiple_of(first_row, _PIECE)
        odd = c % 2
        head = (blk + _SKEW * odd) % _H
        seg = ((rnd + odd) & 1) + (head * _SEGS + c - odd)
        pltpu.make_async_copy(
            src.at[seg, pl.ds(first_row, _PIECE)],
            kv[blk].at[pl.ds(c * _PIECE, _PIECE)],
            kv_sem.at[blk],
        ).start(priority=odd)

    def kv_wait(blk):
        pltpu.make_async_copy(kv[blk], kv[blk], kv_sem.at[blk]).wait()

    def kv_tile(blk, t):
        return kv[blk][pl.ds(t * _LANES, _LANES)]

    def w_copy(src, dst, sem, r, c, rows=_WROWS, cols=_WCOLS):
        where = (pl.ds(r, rows), pl.ds(c, cols))
        return pltpu.make_async_copy(src.at[where], dst.at[where], sem)

    def step(start, first, tasks, pieces=_SEGS):
        for part in range(4):
            for p in range(pieces * part // 4, pieces * (part + 1) // 4):
                start(first + p + _AHEAD)
            for task in tasks[part::4]:
                task()

    def share(tasks):
        return lambda blk: tasks[len(tasks) * blk // _H:len(tasks) * (blk + 1) // _H]

    row = lax.broadcasted_iota(jnp.int32, (_H, _LANES), 0)
    col = lax.broadcasted_iota(jnp.int32, (_H, _LANES), 1)
    row_dh = lax.broadcasted_iota(jnp.int32, (_H, _DH), 0)
    owner = (row - _SKEW * ((col >> (_PIECE.bit_length() - 1)) & 1)) & (_H - 1)

    wq_pieces = [(_WROWS * p, _WCOLS * g) for g in range(w_groups) for p in _spread(w_tiles)]

    def wq_copy(n):
        return w_copy(wq_hbm, wq, wq_sem.at[n // _SEGS], *wq_pieces[n])

    def start_wq_then_k(n):
        if n < len(wq_pieces):
            wq_copy(n).start(priority=n % 2)
        else:
            kv_start(k_hbm, 0, n - len(wq_pieces))

    def start_wq_pair(i, _):
        for odd in range(2):
            n = 2 * i + odd
            g, p = lax.div(n, w_tiles), lax.rem(n, w_tiles)
            r = lax.div(p, w_tiles // 8) + 8 * lax.rem(p, w_tiles // 8)
            w_copy(wq_hbm, wq, wq_sem.at[lax.div(n, _SEGS)],
                   pl.multiple_of(r * _WROWS, _WROWS),
                   pl.multiple_of(g * _WCOLS, _WCOLS)).start(priority=odd)

    x_copy = pltpu.make_async_copy(x_hbm, x_ref, misc_sem.at[0])
    b1_copy = pltpu.make_async_copy(b1_hbm, b1_ref, misc_sem.at[1])
    x_copy.start()
    b1_copy.start()
    for n in range(_BURST):
        start_wq_then_k(n)
    lax.fori_loop(_BURST // 2, _AHEAD // 2, start_wq_pair, None)
    x_copy.wait()
    b1_copy.wait()
    x = x_ref[0].astype(f32)
    centered = x - jnp.mean(x, axis=-1, keepdims=True)
    var = jnp.mean(centered * centered, axis=-1, keepdims=True)
    xn = jnp.broadcast_to(centered * lax.rsqrt(var + _EPS), (_H, d)).astype(bf16)

    q = [jnp.zeros((_H, _DH), f32)]

    def project_q(h):
        q[0] = jnp.where(row_dh == h, _dot(xn, wq[:, _DH * h:_DH * (h + 1)]), q[0])

    done = 0
    for first in range(0, len(wq_pieces), _SEGS):
        for n in range(first, first + _SEGS):
            wq_copy(n).wait()
        landed = heads_per_group * ((first + _SEGS) // w_tiles)
        upto = landed if landed == _H else min(landed, done + 2)
        step(start_wq_then_k, first, [lambda h=h: project_q(h) for h in range(done, upto)])
        done = upto
    q_ref[...] = q[0].astype(bf16)

    lowest = jnp.full((_H, _LANES), -jnp.inf, f32)

    def score_round(rnd, running_max, start, extra=lambda blk: []):
        s = [lowest] * _TILES
        for blk in range(_H):
            kv_wait(blk)
            qs = q_ref[...]

            def tile(t):
                s[t] = jnp.where(owner == blk, _dot_nt(qs, kv_tile(blk, t)), s[t])

            step(start, blk * _SEGS, [lambda t=t: tile(t) for t in range(_TILES)] + extra(blk))
        for t in range(_TILES):
            scores[rnd, t] = s[t]
            running_max = jnp.maximum(running_max, s[t])
        return running_max

    def start_mlp_weights(n):
        r = pl.multiple_of(lax.shift_right_logical(n, 1) * _WROWS, _WROWS)
        c = pl.multiple_of((n & 1) * (ff // 2), _LANES)
        w_copy(w1_hbm, w1, misc_sem.at[0], r, c, cols=ff // 2).start(priority=1)
        w_copy(w2t_hbm, w2t, misc_sem.at[1], r, c, cols=ff // 2).start(priority=1)

    mlp_rounds = 2 * w_tiles // _H
    running_max = lax.fori_loop(
        0, mlp_rounds,
        lambda rnd, m: score_round(
            rnd, m, lambda n: kv_start(k_hbm, rnd, n),
            lambda blk: [lambda: start_mlp_weights(rnd * _H + blk)]),
        lowest)
    running_max = lax.fori_loop(
        mlp_rounds, last_round,
        lambda rnd, m: score_round(rnd, m, lambda n: kv_start(k_hbm, rnd, n)),
        running_max)
    pltpu.make_async_copy(w1, w1, misc_sem.at[0]).wait()
    pltpu.make_async_copy(w2t, w2t, misc_sem.at[1]).wait()

    hidden = [jnp.zeros((_H, _LANES), f32)]

    def mlp_in(c):
        h = _dot(xn, w1[:, _LANES * c:_LANES * (c + 1)])
        hidden[0] = jnp.where(row == c, h, hidden[0])

    def start_k_then_v(n):
        if n < _ROUND:
            kv_start(k_hbm, last_round, n)
        else:
            kv_start(v_hbm, 0, n - _ROUND)

    running_max = score_round(
        last_round, running_max, start_k_then_v,
        share([lambda c=c: mlp_in(c) for c in range(ff // _LANES)]))
    row_max = jnp.max(running_max, axis=1, keepdims=True)

    bias = jnp.concatenate(
        [b1_ref[...].astype(f32), jnp.zeros((_H - ff // _LANES, _LANES), f32)], axis=0)
    pre = hidden[0] + bias
    softplus = jnp.log1p(jnp.exp(-jnp.abs(pre))) + jnp.where(pre > 0, pre, 0.0)
    act = pre * jnp.tanh(softplus)

    def value_round(rnd, carry, start, extra=lambda blk: []):
        denom, acc = carry[0], [carry[1]]
        e = [jnp.exp((scores[rnd, t] - row_max) * (_DH ** -0.5)) for t in range(_TILES)]
        for blk in range(_H):
            kv_wait(blk)

            def tile(t):
                p = jnp.where(owner == blk, e[t], 0.0).astype(bf16)
                acc[0] = acc[0] + _dot(p, kv_tile(blk, t))

            step(start, blk * _SEGS, [lambda t=t: tile(t) for t in range(_TILES)] + extra(blk))
        return sum(e, denom), acc[0]

    row_blocks = [(r, min(_LANES, d - r)) for r in range(0, d, _LANES)]
    wo_units = []
    for g in range(w_groups):
        if g < w_groups // 2:
            pieces = [(_WROWS * p, _WCOLS * g) for p in _spread(w_tiles)]
            wo_units += [(pieces[:16], None, []), (pieces[16:32], None, []),
                         (pieces[32:], None, [(g, i) for i in range(len(row_blocks))])]
            continue
        for blocks in ([0], [1], [2, 3]) if g < w_groups - 1 else ([0], [1], [2], [3]):
            pieces = [(row_blocks[i][0] + _WROWS * p, _WCOLS * g)
                      for i in blocks for p in _spread(row_blocks[i][1] // _WROWS)]
            region = (row_blocks[blocks[0]][0], _WCOLS * g, _WROWS * len(pieces))
            wo_units.append((pieces, region, [(g, i) for i in blocks]))
    wo_pieces = [(u, piece) for u, unit in enumerate(wo_units) for piece in unit[0]]

    def start_v_then_wo(n):
        if n < _ROUND:
            kv_start(v_hbm, last_round, n)
        elif n < _ROUND + len(wo_pieces):
            u, piece = wo_pieces[n - _ROUND]
            late = n >= _ROUND + len(wo_pieces) - _DRAIN
            w_copy(wot_hbm, wot, wo_sem.at[u], *piece).start(priority=1 if late else n % 2)

    mlp = [jnp.zeros((_H, d), f32)]

    def mlp_out(c):
        lhs = jnp.where(row == c, act, 0.0).astype(bf16)
        mlp[0] = mlp[0] + _dot_nt(lhs, w2t[:, _LANES * c:_LANES * (c + 1)])

    carry = lax.fori_loop(
        0, last_round,
        lambda rnd, c: value_round(rnd, c, lambda n: kv_start(v_hbm, rnd, n)),
        (jnp.zeros((_H, _LANES), f32), jnp.zeros((_H, _DH), f32)))
    denom, acc = value_round(
        last_round, carry, start_v_then_wo,
        share([lambda c=c: mlp_out(c) for c in range(ff // _LANES)]))

    attn = acc / jnp.sum(denom, axis=1, keepdims=True)
    attn_rows = [
        jnp.concatenate(
            [jnp.broadcast_to(attn[h:h + 1], (_H, _DH))
             for h in range(heads_per_group * g, heads_per_group * (g + 1))],
            axis=1).astype(bf16)
        for g in range(w_groups)]
    base = x + jnp.sum(mlp[0], axis=0, keepdims=True)
    out = [base[:, r:r + n] for r, n in row_blocks]

    def project_out(g, i):
        r, n = row_blocks[i]
        out[i] = out[i] + _dot_nt(attn_rows[g], wot[r:r + n, _WCOLS * g:_WCOLS * (g + 1)])[:1]

    first, todo = _ROUND, []
    for u, (pieces, region, unlocked) in enumerate(wo_units):
        if region is None:
            for piece in pieces:
                w_copy(wot_hbm, wot, wo_sem.at[u], *piece).wait()
        else:
            w_copy(wot_hbm, wot, wo_sem.at[u], *region).wait()
        todo += unlocked
        now, todo = todo[:3], todo[3:]
        step(start_v_then_wo, first, [lambda a=a: project_out(*a) for a in now], len(pieces))
        first += len(pieces)
    assert not todo

    out_ref[0] = jnp.concatenate(out, axis=1).astype(out_ref.dtype)
    out_copy = pltpu.make_async_copy(out_ref, out_hbm, misc_sem.at[0])
    out_copy.start()
    out_copy.wait()


@jax.jit
def pallas_parallel_sum__mha_block_cached__dense_activation_mish__decode_kernel(
    A_x: jax.Array,
    A_k_cache: jax.Array,
    A_v_cache: jax.Array,
    A_wq: jax.Array,
    A_wo: jax.Array,
    B_x: jax.Array,
    B_w1: jax.Array,
    B_b1: jax.Array,
    B_w2: jax.Array,
):
    del B_x
    d, ff = B_w1.shape
    seg_rows = A_k_cache.shape[2] // _SEGS
    dtype = A_x.dtype
    hbm = pl.BlockSpec(memory_space=pltpu.HBM)
    return pl.pallas_call(
        _kernel,
        out_shape=jax.ShapeDtypeStruct(A_x.shape, dtype),
        in_specs=[hbm] * 8,
        out_specs=hbm,
        scratch_shapes=[
            [pltpu.VMEM((_SEGS * _PIECE, _DH), dtype) for _ in range(_H)],
            pltpu.VMEM((seg_rows // _PIECE, _TILES, _H, _LANES), jnp.float32),
            pltpu.VMEM((_H, _DH), jnp.bfloat16),
            pltpu.VMEM((d, _H * _DH), dtype),
            pltpu.VMEM((d, _H * _DH), dtype),
            pltpu.VMEM((d, ff), dtype),
            pltpu.VMEM((d, ff), dtype),
            pltpu.VMEM(A_x.shape, dtype),
            pltpu.VMEM((ff // _LANES, _LANES), dtype),
            pltpu.VMEM(A_x.shape, dtype),
            pltpu.SemaphoreType.DMA((_H,)),
            pltpu.SemaphoreType.DMA((14,)),
            pltpu.SemaphoreType.DMA((13,)),
            pltpu.SemaphoreType.DMA((2,)),
        ],
        compiler_params=pltpu.CompilerParams(
            vmem_limit_bytes=32 * 2**20,
            disable_bounds_checks=True,
            disable_semaphore_checks=True,
        ),
    )(
        A_x,
        A_k_cache.reshape(_ROUND, seg_rows, _DH),
        A_v_cache.reshape(_ROUND, seg_rows, _DH),
        A_wq,
        A_wo.T,
        B_w1,
        B_b1.reshape(ff // _LANES, _LANES),
        B_w2.T,
    )
```
